```python
import jax
import jax.numpy as jnp

def _softmax(x, axis=-1):
    return jax.nn.softmax(x, axis=axis)
def _gelu(x):
    return jax.nn.gelu(x, approximate=True)
def _silu(x):
    return jax.nn.silu(x)
def _sigmoid(x):
    return jax.nn.sigmoid(x)
def _layernorm(x, axis=-1, eps=1e-5):
    m = jnp.mean(x, axis=axis, keepdims=True)
    v = jnp.var(x, axis=axis, keepdims=True)
    return (x - m) / jnp.sqrt(v + eps)
def _scatter_add(tgt, idx, src, axis=0):
    return tgt.at[idx].add(src)
def _segment_sum(src, seg, n):
    return jax.ops.segment_sum(src, seg, n)
class _Rng:
    def __init__(self, key):
        self._k = key
    def _next(self):
        self._k, sub = jax.random.split(self._k)
        return sub
    def normal(self, shape):
        return jax.random.normal(self._next(), shape, dtype=jnp.bfloat16)
    def randint(self, lo, hi, shape):
        return jax.random.randint(self._next(), shape, lo, hi, dtype=jnp.int32)
    def uniform(self, shape, lo=0.0, hi=1.0):
        return jax.random.uniform(self._next(), shape, jnp.bfloat16, lo, hi)
    def permutation(self, n):
        return jax.random.permutation(self._next(), n)


kernel_name = 'standalone__mha_softmax__near_ridge'

def _fwd_setup_inputs():
    _rng = _Rng(jax.random.key(int.from_bytes(__import__("os").urandom(4), "little")))
    _w = (lambda a: (lambda t: t.astype(jnp.bfloat16) if jnp.issubdtype(t.dtype, jnp.floating) else t)(jnp.asarray(a)))
    B, H, Sq, Sk, D = 16, 32, 384, 1024, 128
    return {
        "q": _w((lambda *s: _rng.normal(s) * 0.05)(B, H, Sq, D)),
        "k": _w((lambda *s: _rng.normal(s) * 0.05)(B, H, Sk, D)),
        "v": _w((lambda *s: _rng.normal(s) * 0.05)(B, H, Sk, D)),
    }

def _fwd_reference(q, k, v):
    scale = q.shape[-1] ** -0.5
    scores = jnp.einsum("bhqd,bhkd->bhqk", q, k) * scale
    p = _softmax(scores, axis=-1)
    return jnp.einsum("bhqk,bhkd->bhqd", p, v)


def setup_inputs():
    _inp = _fwd_setup_inputs()
    _gk = jax.random.fold_in(jax.random.key(int.from_bytes(__import__("os").urandom(4), "little")), 2**31 - 1)
    _shapes = [[16, 32, 384, 128]]
    _dtypes = ['bfloat16']
    _gks = jax.random.split(_gk, len(_shapes))
    _gs = [jax.random.normal(k, s, dtype=jnp.dtype(d)) * 0.05 for k, s, d in zip(_gks, _shapes, _dtypes)]
    _inp["grad_out"] = _gs[0]
    return _inp

def reference(q, k, v, grad_out):
    _const = dict()
    def _f(*_d):
        return _fwd_reference(**{'q': _d[0], 'k': _d[1], 'v': _d[2], **_const})
    _out, _vjp = jax.vjp(_f, q, k, v)
    _grads = _vjp(grad_out)
    _out0 = jnp.asarray(_out)
    return (_out0, *[jnp.asarray(_g) for _g in _grads])
```

```python
import functools, math
import jax, jax.numpy as jnp
from jax.experimental import pallas as pl
from jax.experimental.pallas import tpu as pltpu
NT = (((1,), (1,)), ((), ()))
NN = (((1,), (0,)), ((), ()))
f32 = jnp.float32; bf16 = jnp.bfloat16; u32 = jnp.uint32
def dot(a, b, dims=NN): return jax.lax.dot_general(a, b, dims, preferred_element_type=f32)
T = 128
ORDERS = {
 "a": "A0 A1 V0 B0 C0 A2 B1 N0 E0 C1 D0 K0 B2 N1 G0 H0 E1 C2 D1 N2 G1 H1 D2 E2 H2 G2",
 "b": "A0 A1 V0 B0 A2 C0 B1 N0 C1 E0 D0 B2 K0 N1 C2 E1 G0 H0 D1 N2 D2 G1 H1 E2 H2 G2",
}
def make(hb=1, order="a", R=256, bc=1, lp=0, fold=0):
    order = ORDERS.get(order, order).replace("_", " ").split()
    def kern(q_ref, k_ref, v_ref, do_ref, o_ref, dq_ref, dk_ref, dv_ref, kT_scr, vT_scr, p_scr, ds_scr):
        Sq, D = q_ref.shape[1:]; Sk = k_ref.shape[1]
        nq = Sq // T; nk = Sk // T; nr = Sk // R; rt = R // T
        scale = D ** -0.5; c = scale * math.log2(math.e)
        def ld(ref, h, a, n):
            if bc:
                return pltpu.bitcast(ref.bitcast(u32)[h, a//2:(a+n)//2, :], bf16)
            return ref[h, a:a+n, :]
        pk = lambda x: pltpu.bitcast(x.astype(bf16), u32)
        upk = lambda x: pltpu.bitcast(x, bf16)
        def head(h):
            st = {}
            jj = lambda j: (h % 2) * nq + j
            def A(j):
                qj = ld(q_ref, h, j*T, T)
                if fold: qj = (qj.astype(f32) * c).astype(bf16)
                mx = None
                for u in range(nr):
                    s = dot(ld(k_ref, h, u*R, R), qj, NT)
                    for t in range(rt): st["s", j, u*rt+t] = s[t*T:(t+1)*T]
                    mu = jnp.max(s.reshape(R // 8, 8, T), axis=0)
                    mx = mu if mx is None else jnp.maximum(mx, mu)
                st["m", j] = jnp.max(mx, axis=0, keepdims=True)
            def Vt(_):
                for u in range(nk): vT_scr[u] = pltpu.bitcast(ld(v_ref, h, u*T, T).T, u32)
            def Kt(_):
                for u in range(nk): kT_scr[u] = pltpu.bitcast(ld(k_ref, h, u*T, T).T, u32)
            def B(j):
                m = st["m", j]; ls = None
                for u in range(nk):
                    x = st["s", j, u] - m
                    p = jnp.exp2(x if fold else x * c)
                    p_scr[jj(j), u*T:(u+1)*T, :] = p.astype(bf16)
                    if lp: p = ld(p_scr, jj(j), u*T, T).astype(f32)
                    lu = jnp.sum(p.reshape(T // 8, 8, T), axis=0)
                    ls = lu if ls is None else ls + lu
                r = 1.0 / jnp.sum(ls, axis=0, keepdims=True)
                st["r", j] = r
                doT = do_ref[h, j*T:(j+1)*T, :].astype(f32).T
                st["doT", j] = doT
                st["do1", j] = (doT * r).astype(bf16)
                st["do2", j] = (doT * (r * scale)).astype(bf16)
            def cat(name, j, u): return ld(dict(p=p_scr, ds=ds_scr)[name], jj(j), u*R, R)
            def C(j):
                acc = None
                for u in range(nk):
                    x = dot(pltpu.bitcast(vT_scr[u], bf16), ld(p_scr, jj(j), u*T, T))
                    acc = x if acc is None else acc + x
                st["oT", j] = acc
            def N(j):
                r = st["r", j]
                oT = st["oT", j] * r
                o_ref[h, j*T:(j+1)*T, :] = oT.T.astype(bf16)
                st["delta", j] = jnp.sum(oT * st["doT", j], axis=0, keepdims=True) * (r * scale)
            def Dd(j):
                for u in range(nr):
                    dp = dot(ld(v_ref, h, u*R, R), st["do2", j])
                    pf = cat("p", j, u).astype(f32)
                    ds_scr[jj(j), u*R:(u+1)*R, :] = (pf * (dp - st["delta", j])).astype(bf16)
            def accum(name, out, j, u, x):
                if j > 0: x = x + st[name, u]
                st[name, u] = x
                if j == nq - 1: out[h, u*R:(u+1)*R, :] = x.astype(bf16)
            def E(j):
                for u in range(nr):
                    accum("dv", dv_ref, j, u, dot(cat("p", j, u), st["do1", j], NT))
            def G(j):
                qj = ld(q_ref, h, j*T, T)
                for u in range(nr):
                    accum("dk", dk_ref, j, u, dot(cat("ds", j, u), qj))
            def H(j):
                acc = None
                for u in range(nk):
                    x = dot(pltpu.bitcast(kT_scr[u], bf16), ld(ds_scr, jj(j), u*T, T))
                    acc = x if acc is None else acc + x
                dq_ref[h, j*T:(j+1)*T, :] = acc.T.astype(bf16)
            fns = dict(A=A, V=Vt, K=Kt, B=B, C=C, N=N, D=Dd, E=E, G=G, H=H)
            for o in order:
                fns[o[0]](int(o[1]))
        for h in range(hb): head(h)

    @jax.jit
    def mha(q, k, v, do):
        B, H, Sq, D = q.shape; Sk = k.shape[2]; nq = Sq // T
        r3 = lambda x: x.reshape(B * H, *x.shape[2:])
        qs = pl.BlockSpec((hb, Sq, D), lambda i: (i, 0, 0)); ks = pl.BlockSpec((hb, Sk, D), lambda i: (i, 0, 0))
        outs = pl.pallas_call(kern, grid=(B * H // hb,), in_specs=[qs, ks, ks, qs], out_specs=[qs, qs, ks, ks],
            out_shape=[jax.ShapeDtypeStruct((B * H, Sq, D), bf16)] * 2 + [jax.ShapeDtypeStruct((B * H, Sk, D), bf16)] * 2,
            scratch_shapes=[pltpu.VMEM((Sk // T, D // 2, T), u32), pltpu.VMEM((Sk // T, D // 2, T), u32), pltpu.VMEM((2 * nq, Sk, T), bf16), pltpu.VMEM((2 * nq, Sk, T), bf16)],
            compiler_params=pltpu.CompilerParams(dimension_semantics=("parallel",), vmem_limit_bytes=100 * 2**20))(r3(q), r3(k), r3(v), r3(do))
        return tuple(o.reshape(B, H, *o.shape[1:]) for o in outs)
    return mha


_mha = make(hb=4, order="b", lp=1, fold=1)


@jax.jit
def pallas_standalone__mha_softmax__near_ridge_kernel(q: jax.Array, k: jax.Array, v: jax.Array, grad_out: jax.Array):
    return _mha(q, k, v, grad_out)
```

```python
import functools, math
import jax, jax.numpy as jnp
from jax.experimental import pallas as pl
from jax.experimental.pallas import tpu as pltpu
NT = (((1,), (1,)), ((), ()))
NN = (((1,), (0,)), ((), ()))
f32 = jnp.float32; bf16 = jnp.bfloat16; u32 = jnp.uint32
def dot(a, b, dims=NN): return jax.lax.dot_general(a, b, dims, preferred_element_type=f32)
T = 128
NB = 3

def schedule(nheads, pat, pro, epi):
    toks = []
    for h in range(nheads):
        p = pro if h == 0 else pat
        toks += [(t[0], 3 * h + int(t[1:])) for t in p.split("_") if t]
    toks += [(t[0], 3 * (nheads - 1) + int(t[1:])) for t in epi.split("_") if t]
    return toks

def make(hb=2, pat="A0_H-1_B0_Y-3_A1_C0_B1_N0_A2_C1_B2_N1_D0_C2_N2_D1_X0_H0_D2_H1", pro="A0_A1_B0_A2_B1_C0_B2_N0_C1_N1_D0_C2_N2_D1_X0_H0_D2_H1", R=256, lp=1, fold=0, pace=1, bc=1, verbose=0, epi="H2_Y0", r=4, sb=1, nobc=1, nolmr=0, tie=2, tb=2):
    class V:
        def __init__(s, ref, base): s.r = ref; s.base = base; s.shape = ref.shape
        def bitcast(s, t): return V(s.r.bitcast(t), s.base)
        def __getitem__(s, i): return s.r[(s.base + i[0],) + i[1:]]
        def __setitem__(s, i, x): s.r[(s.base + i[0],) + i[1:]] = x
    ns = r // sb
    def kern(*refs):
        in_hbm, out_hbm = refs[0:4], refs[4:8]
        in_big, out_big, in_sm, out_sm = refs[8:12], refs[12:16], refs[16:20], refs[20:24]
        sem_ib, sem_ob, sem_is, sem_os = refs[24:28]
        scr = refs[28:]
        nh = in_hbm[0].shape[0]; nb = (nh - 2 * r) // hb
        step = pl.program_id(0)
        def cp_in(bufs, sems, s, pos, g, n): return [pltpu.make_async_copy(a.at[pl.ds(g, n)], b.at[pl.ds(pos, n)], sems.at[s, i]) for i, (a, b) in enumerate(zip(in_hbm, bufs))]
        def cp_out(bufs, sems, s, pos, g, n): return [pltpu.make_async_copy(b.at[pl.ds(pos, n)], a.at[pl.ds(g, n)], sems.at[s, i]) for i, (a, b) in enumerate(zip(out_hbm, bufs))]
        phase = step
        @pl.when(phase == 0)
        def _():
            for c_ in cp_in(in_sm, sem_is, 0, 0, 0, sb): c_.start()
            for c_ in cp_in(in_sm, sem_is, 0, 0, 0, sb): c_.wait()
            for x in range(1, ns):
                for c_ in cp_in(in_sm, sem_is, x, x * sb, x * sb, sb): c_.start()
            for c_ in cp_in(in_big, sem_ib, 0, 0, r, hb): c_.start()
        def small(i, carry):
            @pl.when(i > 0)
            def _():
                for c_ in cp_in(in_sm, sem_is, i, i * sb, 0, sb): c_.wait()
            scoped(sb, [V(x, i * sb) for x in in_sm + out_sm])
            @pl.when(phase == 1)
            def _():
                for c_ in cp_out(out_sm, sem_os, i, i * sb, nh - 2 * r + i * sb, sb): c_.start()
            return carry
        jax.lax.fori_loop(phase * ns, phase * ns + ns, small, 0)
        @pl.when(phase == 0)
        def _():
            for c_ in cp_in(in_big, sem_ib, 0, 0, 0, hb): c_.wait()
            for c_ in cp_in(in_big, sem_ib, 1, hb, r + hb, hb): c_.start()
            for x in range(ns):
                for c_ in cp_out(out_sm, sem_os, x, x * sb, x * sb, sb): c_.start()
            for x in range(ns, 2 * ns):
                for c_ in cp_in(in_sm, sem_is, x, x * sb, nh - 2 * r + x * sb, sb): c_.start()
            def big(b, carry):
                half = b & 1
                @pl.when(b >= 2)
                def _():
                    for c_ in cp_out(out_big, sem_ob, half, half * hb, 0, hb): c_.wait()
                @pl.when(b >= 1)
                def _():
                    for c_ in cp_in(in_big, sem_ib, half, half * hb, 0, hb): c_.wait()
                scoped(hb, [V(x, half * hb) for x in in_big + out_big])
                @pl.when(b + 2 < nb)
                def _():
                    for c_ in cp_in(in_big, sem_ib, half, half * hb, r + (b + 2) * hb, hb): c_.start()
                for c_ in cp_out(out_big, sem_ob, half, half * hb, r + b * hb, hb): c_.start()
                return carry
            jax.lax.fori_loop(0, nb, big, 0)
        @pl.when(phase == 1)
        def _():
            for x in range(2):
                for c_ in cp_out(out_big, sem_ob, x, x * hb, 0, hb): c_.wait()
            for x in range(2 * ns):
                for c_ in cp_out(out_sm, sem_os, x, x * sb, 0, sb): c_.wait()

    def scoped(nheads, views):
        Sk, D = views[1].shape[1:]
        pl.run_scoped(lambda *scr: block(nheads, *views, *scr),
            pltpu.VMEM((2, Sk // T, D // 2, T), u32), pltpu.VMEM((2, Sk // T, D // 2, T), u32), pltpu.VMEM((NB, Sk, T), bf16), pltpu.VMEM((NB, Sk, T), bf16))

    def block(nheads, q_ref, k_ref, v_ref, do_ref, o_ref, dq_ref, dk_ref, dv_ref, kT_scr, vT_scr, p_scr, ds_scr):
        Sq, D = q_ref.shape[1:]; Sk = k_ref.shape[1]
        nq = Sq // T; nk = Sk // T; nr = Sk // R; rt = R // T
        scale = D ** -0.5; c = scale * math.log2(math.e)
        never = pl.program_id(0) < 0
        def ld(ref, h, a, n):
            if bc: return pltpu.bitcast(ref.bitcast(u32)[h, a//2:(a+n)//2, :], bf16)
            return ref[h, a:a+n, :]
        st = {}
        tr = (lambda x: x.astype(bf16).T) if tb else (lambda x: x.T.astype(bf16))
        def xp(ref, h, u):
            y = pltpu.bitcast(ld(ref, h, u*T, T).T, u32)
            return jnp.where(never, jnp.zeros_like(y), y) if nolmr else y
        pend = []
        def outT(ref, h, j, x):
            if tb == 2:
                y = pltpu.bitcast(x.astype(bf16).T, u32)
                ref.bitcast(u32)[h, j*T//2:(j+1)*T//2, :] = y
                pend.append([len(taps), pltpu.bitcast(y[T//2-8:], f32)])
            else:
                y = x.T
                ref[h, j*T:(j+1)*T, :] = y.astype(bf16)
                pend.append([len(taps), y[T-8:]])
        def tied(x):
            while tie and pend and pend[0][0] + tie <= len(taps):
                x = jnp.where(never, pend.pop(0)[1][:x.shape[0]], x)
            return x
        taps = []
        def tap4(xs): taps.append([xs[0][(xs[0].shape[0] // 8) * i:(xs[0].shape[0] // 8) * i + 8] for i in range(8)])
        def tap8(xs): taps.append([xs[4 * (i // 4)][32 * (i % 4):32 * (i % 4) + 8] for i in range(8)])
        def A(t, R=R, nr=nr, rt=rt):
            h, j = divmod(t, nq)
            qj = ld(q_ref, h, j*T, T)
            if fold: qj = (qj.astype(f32) * c).astype(bf16)
            mx = None; xs = []
            for u in range(nr):
                s = dot(ld(k_ref, h, u*R, R), qj, NT); xs.append(s)
                for i in range(rt): st["s", t, u*rt+i] = s[i*T:(i+1)*T]
                mu = jnp.max(s.reshape(R // 8, 8, T), axis=0)
                mx = mu if mx is None else jnp.maximum(mx, mu)
            st["m", t] = jnp.broadcast_to(jnp.max(mx, axis=0, keepdims=True), (8, T))
            tap4(xs)
        def B(t):
            h, j = divmod(t, nq)
            m = tied(st["m", t]); ls = None
            tp = taps[-1] if pace == 1 else taps[-2][::2] + taps[-1][::2]
            for u in range(nk):
                mu = jnp.where(never, tp[u], m) if pace else m
                x = (st["s", t, u].reshape(T // 8, 8, T) - mu[None]).reshape(T, T)
                p = jnp.exp2(x if fold else x * c)
                p_scr[t % NB, u*T:(u+1)*T, :] = p.astype(bf16)
                if lp: p = ld(p_scr, t % NB, u*T, T).astype(f32)
                lu = jnp.sum(p.reshape(T // 8, 8, T), axis=0)
                ls = lu if ls is None else ls + lu
            r = 1.0 / jnp.sum(ls, axis=0, keepdims=True)
            st["r", t] = r
            doT = do_ref[h, j*T:(j+1)*T, :].astype(f32).T
            st["doT", t] = doT
            st["do1", t] = (doT * r).astype(bf16)
            st["do2", t] = (doT * (r * scale)).astype(bf16)
        def C(t):
            h, j = divmod(t, nq)
            if j == 0:
                for u in range(nk): vT_scr[h % 2, u] = xp(v_ref, h, u)
            xs = [dot(pltpu.bitcast(vT_scr[h % 2, u], bf16), ld(p_scr, t % NB, u*T, T)) for u in range(nk)]
            st["oT", t] = functools.reduce(jnp.add, xs)
            tap8(xs)
        def N(t):
            h, j = divmod(t, nq)
            r = st["r", t]
            oT = st["oT", t] * r
            outT(o_ref, h, j, oT)
            st["delta", t] = jnp.sum(oT * st["doT", t], axis=0, keepdims=True) * (r * scale)
        def Dd(t, R=R, nr=nr):
            h, j = divmod(t, nq); xs = []
            st["delta", t] = tied(st["delta", t])
            for u in range(nr):
                dp = dot(ld(v_ref, h, u*R, R), st["do2", t]); xs.append(dp)
                pf = ld(p_scr, t % NB, u*R, R).astype(f32)
                ds_scr[t % NB, u*R:(u+1)*R, :] = (pf * (dp - st["delta", t])).astype(bf16)
            tap4(xs)
        def accum(name, out, t, xs):
            h, j = divmod(t, nq)
            for u, x in enumerate(xs):
                if j > 0: x = x + st[name, u]
                st[name, u] = x
                if j == nq - 1: out[h, u*R:(u+1)*R, :] = x.astype(bf16)
            tap4(xs)
        def E(t):
            accum("dv", dv_ref, t, [dot(ld(p_scr, t % NB, u*R, R), st["do1", t], NT) for u in range(nr)])
        def G(t):
            h, j = divmod(t, nq)
            qj = ld(q_ref, h, j*T, T)
            accum("dk", dk_ref, t, [dot(ld(ds_scr, t % NB, u*R, R), qj) for u in range(nr)])
        def H(t):
            h, j = divmod(t, nq)
            if j == 0:
                for u in range(nk): kT_scr[h % 2, u] = xp(k_ref, h, u)
            xs = [dot(pltpu.bitcast(kT_scr[h % 2, u], bf16), ld(ds_scr, t % NB, u*T, T)) for u in range(nk)]
            outT(dq_ref, h, j, functools.reduce(jnp.add, xs))
            tap8(xs)
        def EG(h, isE, RR):
            ws = [st["do1", nq*h+j] if isE else ld(q_ref, h, j*T, T) for j in range(nq)]
            scr, out = (p_scr, dv_ref) if isE else (ds_scr, dk_ref)
            res = []
            for u in range(Sk // RR):
                xs = [dot(ld(scr, (nq*h+j) % NB, u*RR, RR), ws[j], NT if isE else NN) for j in range(nq)]
                out[h, u*RR:(u+1)*RR, :] = functools.reduce(jnp.add, xs).astype(bf16)
                res.append(xs[0])
            return res
        def X(t): taps.append([x[:8] for x in EG(t // nq, True, T)])
        def Y(t): taps.append([x[:8] for x in EG(t // nq, False, T)])
        def U(t): EG(t // nq, True, Sk); Dd(t, Sk, 1)
        def W(t): EG(t // nq - 1, False, Sk); A(t, Sk, 1, Sk // T)
        fns = dict(X=X, Y=Y, U=U, W=W, A=A, B=B, C=C, N=N, D=Dd, E=E, G=G, H=H)
        toks = schedule(nheads, pat, pro, epi)
        if verbose: print(" ".join(f"{a}{b}" for a, b in toks))
        for a, b in toks: fns[a](b)

    @jax.jit
    def mha(q, k, v, do):
        B, H, Sq, D = q.shape; Sk = k.shape[2]; nq = Sq // T
        r3 = lambda x: x.reshape(B * H, *x.shape[2:])
        qs = ks = pl.BlockSpec(memory_space=pl.ANY)
        assert (B * H - 2 * r) % hb == 0 and (B * H - 2 * r) // hb >= 2
        def bufs(n):
            qb = pltpu.VMEM((n, Sq, D), bf16); kb = pltpu.VMEM((n, Sk, D), bf16)
            return [qb, kb, kb, qb, qb, qb, kb, kb]
        sems = lambda n: pltpu.SemaphoreType.DMA((n, 4))
        outs = pl.pallas_call(kern, grid=(2,), in_specs=[qs, ks, ks, qs], out_specs=[qs, qs, ks, ks],
            out_shape=[jax.ShapeDtypeStruct((B * H, Sq, D), bf16)] * 2 + [jax.ShapeDtypeStruct((B * H, Sk, D), bf16)] * 2,
            scratch_shapes=bufs(2 * hb) + bufs(2 * r) + [sems(2), sems(2), sems(2 * ns), sems(2 * ns)],
            compiler_params=pltpu.CompilerParams(dimension_semantics=("arbitrary",), vmem_limit_bytes=100 * 2**20, disable_bounds_checks=bool(nobc)))(r3(q), r3(k), r3(v), r3(do))
        return tuple(o.reshape(B, H, *o.shape[1:]) for o in outs)
    return mha


_mha = make(hb=8)


@jax.jit
def pallas_standalone__mha_softmax__near_ridge_kernel(q: jax.Array, k: jax.Array, v: jax.Array, grad_out: jax.Array):
    return _mha(q, k, v, grad_out)
```

```python
import functools
import math

import jax
import jax.numpy as jnp
from jax.experimental import pallas as pl
from jax.experimental.pallas import tpu as pltpu

f32, bf16, u32 = jnp.float32, jnp.bfloat16, jnp.uint32
NN = (((1,), (0,)), ((), ()))
NT = (((1,), (1,)), ((), ()))
T = 128
R = 256
NB = 6


def _dot(a, b, dims=NN):
    return jax.lax.dot_general(a, b, dims, preferred_element_type=f32)


class _Heads:
    def __init__(self, ref, slot):
        self.ref, self.slot, self.shape = ref, slot, ref.shape

    def bitcast(self, dtype):
        return _Heads(self.ref.bitcast(dtype), self.slot)

    def __getitem__(self, i):
        return self.ref[(self.slot(i[0]),) + i[1:]]

    def __setitem__(self, i, x):
        self.ref[(self.slot(i[0]),) + i[1:]] = x


def make(hb=8, r=4, pg=32, tie=2, nm=0, lv=1, so=24,
         pat="F0_F1_F2_C0_N0_C1_N1_C2_N2_D0_D1_X0_D2_A3_H0_B3_A4_H1_B4_A5_Z3_H2_B5_Y0",
         first="A0_A1_B0_A2_B1_Z0_B2",
         last="F0_F1_F2_C0_N0_C1_N1_C2_N2_O0_D0_D1_X0_O3_D2_H0_H1_H2_O1_Y0_O2"):
    def block(nheads, order, emit, q_ref, k_ref, v_ref, do_ref, o_ref, dq_ref, dk_ref, dv_ref,
              p_carry, r_carry, vT_carry, kT_scr, vT_scr, p_scr, ds_scr):
        Sq, D = q_ref.shape[1:]
        Sk = k_ref.shape[1]
        nq, nk, nr = Sq // T, Sk // T, Sk // R
        scale = D ** -0.5
        c = scale * math.log2(math.e)
        st = {}

        def ld(ref, h, a, n):
            return pltpu.bitcast(ref.bitcast(u32)[h, a // 2:(a + n) // 2, :], bf16)

        def tile_T(ref, h, u):
            return pltpu.bitcast(ld(ref, h, u * T, T).T, u32)

        def pbuf(t):
            return (p_carry, t % nq) if t < nq or t >= nq * nheads else (p_scr, t % NB)

        never = pl.program_id(0) < 0
        taps, pend = [], []

        def tap(xs):
            g = pg // len(xs)
            taps.append([x[(x.shape[0] // g) * a:(x.shape[0] // g) * a + 8] for x in xs for a in range(g)])

        def tied(x):
            while pend and pend[0][0] + tie <= len(taps):
                x = jnp.where(never, pend.pop(0)[1][:x.shape[0]], x)
            return x

        def store_T(ref, h, j, x):
            y = pltpu.bitcast(x.astype(bf16).T, u32)
            ref.bitcast(u32)[h, j * T // 2:(j + 1) * T // 2, :] = y
            pend.append([len(taps), pltpu.bitcast(y[T // 2 - 8:], f32)])

        def A(t):
            h, j = divmod(t, nq)
            qj = ld(q_ref, h, j * T, T)
            mx, xs = None, []
            for u in range(nr):
                s = _dot(ld(k_ref, h, u * R, R), qj, NT)
                xs.append(s)
                for i in range(R // T):
                    st["s", t, u * (R // T) + i] = s[i * T:(i + 1) * T]
                mu = jnp.max(s.reshape(R // 8, 8, T), axis=0)
                mx = mu if mx is None else jnp.maximum(mx, mu)
            st["m", t] = jnp.broadcast_to(jnp.max(mx, axis=0, keepdims=True), (8, T))
            tap(xs[:1])

        def B(t):
            m, ls, tp = tied(st["m", t]), None, taps[-1]
            g = pg // nk
            rows = T // g
            buf, slot = pbuf(t)
            for u in range(nk):
                x = jnp.concatenate([
                    (st["s", t, u][a * rows:(a + 1) * rows].reshape(rows // 8, 8, T)
                     - jnp.where(never, tp[u * g + a], m)[None]).reshape(rows, T) for a in range(g)], axis=0)
                buf[slot, u * T:(u + 1) * T, :] = jnp.exp2(x * c).astype(bf16)
                p = ld(buf, slot, u * T, T).astype(f32)
                lu = jnp.sum(p.reshape(T // 8, 8, T), axis=0)
                ls = lu if ls is None else ls + lu
            st["r", t] = 1.0 / jnp.sum(ls, axis=0, keepdims=True)
            if t >= nq * nheads:
                r_carry[t % nq] = jnp.broadcast_to(st["r", t], (8, T))

        def Z(t):
            if t == nq * nheads:
                for u in range(nk):
                    vT_carry[u] = tile_T(v_ref, nheads, u)

        def F(t):
            h, j = divmod(t, nq)
            if h == 0:
                st["r", t] = r_carry[j][:1]
            doT = do_ref[h, j * T:(j + 1) * T, :].astype(f32).T
            st["doT", t] = doT
            st["do1", t] = (doT * st["r", t]).astype(bf16)
            st["do2", t] = (doT * (st["r", t] * scale)).astype(bf16)

        def C(t):
            h, j = divmod(t, nq)
            if j == 0 and h > 0:
                for u in range(nk):
                    vT_scr[h % 2, u] = tile_T(v_ref, h, u)
            xs = [_dot(pltpu.bitcast(vT_scr[h % 2, u] if h else vT_carry[u], bf16), ld(*pbuf(t), u * T, T))
                  for u in range(nk)]
            st["oT", t] = functools.reduce(jnp.add, xs)
            tap(xs[::4])

        def N(t):
            h, j = divmod(t, nq)
            oT = st["oT", t] * st["r", t]
            store_T(o_ref, h, j, oT)
            st["delta", t] = jnp.sum(oT * st["doT", t], axis=0, keepdims=True) * (st["r", t] * scale)

        def Dd(t):
            delta, xs = tied(st["delta", t]), []
            for u in range(nr):
                dp = _dot(ld(v_ref, t // nq, u * R, R), st["do2", t])
                xs.append(dp)
                p = ld(*pbuf(t), u * R, R).astype(f32)
                ds_scr[t % NB, u * R:(u + 1) * R, :] = (p * (dp - delta)).astype(bf16)
            tap(xs[:1])

        def H(t):
            h, j = divmod(t, nq)
            if j == 0:
                for u in range(nk):
                    kT_scr[h % 2, u] = tile_T(k_ref, h, u)
            xs = [_dot(pltpu.bitcast(kT_scr[h % 2, u], bf16), ld(ds_scr, t % NB, u * T, T)) for u in range(nk)]
            store_T(dq_ref, h, j, functools.reduce(jnp.add, xs))
            tap(xs[::4])

        def key_grad(t, out, buf, ws, dims):
            res = []
            for u in range(nk):
                xs = [_dot(ld(*buf(t + j), u * T, T), ws[j], dims) for j in range(nq)]
                out[t // nq, u * T:(u + 1) * T, :] = functools.reduce(jnp.add, xs).astype(bf16)
                res.append(xs[0])
            tap(res)

        def X(t):
            key_grad(t, dv_ref, pbuf, [st["do1", t + j] for j in range(nq)], NT)

        def Y(t):
            key_grad(t, dk_ref, lambda i: (ds_scr, i % NB), [ld(q_ref, t // nq, j * T, T) for j in range(nq)], NN)

        stages = dict(A=A, B=B, C=C, D=Dd, F=F, H=H, N=N, O=emit, X=X, Y=Y, Z=Z)
        for h in range(max(nheads, 1)):
            for tok in order.split("_"):
                stages[tok[0]](nq * h + int(tok[1:]))

    def kernel(*refs):
        in_hbm, out_hbm = refs[0:4], refs[4:8]
        in_big, out_big, in_sm, out_sm = refs[8:12], refs[12:16], refs[16:20], refs[20:24]
        sem_ib, sem_ob, sem_is, sem_os = refs[24:28]
        carry = refs[28:]
        nh, Sk, D = in_hbm[1].shape
        nb = (nh - 2 * r) // hb
        ahead = (1, 1, 1, 0)
        phase = pl.program_id(0)

        def run(nheads, order, views, emit=None):
            pl.run_scoped(lambda *scr: block(nheads, order, emit, *views, *carry, *scr),
                          pltpu.VMEM((2, Sk // T, D // 2, T), u32), pltpu.VMEM((2, Sk // T, D // 2, T), u32),
                          pltpu.VMEM((NB, Sk, T), bf16), pltpu.VMEM((NB, Sk, T), bf16))

        def run_small(nheads, order, slot, i, emit=None):
            run(nheads, order, [_Heads(x, lambda h: slot + h if lv or not h else jnp.minimum(slot + h, 2 * r)) for x in in_sm]
                + [_Heads(x, lambda h: i + h) for x in out_sm], emit)

        def copy(hbm, g, buf, pos, n, sem, out):
            a, b = hbm.at[pl.ds(g, n)], buf.at[pl.ds(pos, n)]
            return pltpu.make_async_copy(b, a, sem) if out else pltpu.make_async_copy(a, b, sem)

        def in_b(b):
            return [copy(in_hbm[i], r + b * hb, in_big[i], (b & 1) * (hb + e), hb + e, sem_ib.at[b & 1, i], False)
                    for i, e in enumerate(ahead)]

        def out_b(b):
            return [copy(out_hbm[i], r + b * hb, out_big[i], (b & 1) * hb, hb, sem_ob.at[b & 1, i], True)
                    for i in range(4)]

        def in_s(s, ph):
            return [copy(in_hbm[i], s + ph * (nh - 2 * r - 1), in_sm[i], s, 1, sem_is.at[s, i], False)
                    for i in range(4)]

        def out_s(s, ph):
            return [copy(out_hbm[i], s + ph * (nh - 2 * r), out_sm[i], s, 1, sem_os.at[s, i], True)
                    for i in range(4)]

        def start(cs):
            for x in cs:
                x.start()

        def wait(cs):
            for x in cs:
                x.wait()

        @pl.when(phase == 0)
        def _():
            cs = [x for s in range(r + 1) for x in in_s(s, 0)] + in_b(0)
            start(cs[:so])
            wait(cs[:3])
            start(cs[so:])
            run_small(0, first, 0, 0)
            wait(cs[3:8])

        pl.when(phase == 1)(lambda: wait(in_s(r + 1, 1)))

        def small(i, _):
            pl.when((i > 0) & (i < 2 * r - 1))(lambda: wait(in_s(i + phase + 1, phase)))
            run_small(1, pat, i + phase, i)
            pl.when(phase == 1)(lambda: start(out_s(i, 1)))
            return 0

        jax.lax.fori_loop(phase * r, phase * (r - lv) + r, small, 0)

        @pl.when(phase == 0)
        def _():
            wait(in_b(0))
            start(in_b(1))
            for s in range(r):
                start(out_s(s, 0))
            for s in range(r + 1, 2 * r + 1):
                start(in_s(s, 1))

            def big(b, _):
                pl.when(b >= 2)(lambda: wait(out_b(b - 2)))
                pl.when(b >= 1)(lambda: wait(in_b(b)))
                run(hb, pat, [_Heads(x, lambda h, e=e: (b & 1) * (hb + e) + h)
                              for x, e in zip(in_big + out_big, ahead + (0,) * 4)])
                pl.when(b + 2 < nb)(lambda: start(in_b(b + 2)))
                start(out_b(b))
                return 0

            jax.lax.fori_loop(0, nb, big, 0)

        @pl.when(phase == 1)
        def _():
            if lv: run_small(1, last, 2 * r, 2 * r - 1, lambda i: out_s(2 * r - 1, 1)[i].start())
            wait(out_b(nb - 2) + out_b(nb - 1))
            for s in range(2 * r):
                wait(out_s(s, s // r))

    @jax.jit
    def mha(q, k, v, do):
        B, H, Sq, D = q.shape
        Sk = k.shape[2]
        assert Sq == 3 * T and r >= 2 and (B * H - 2 * r) % hb == 0 and (B * H - 2 * r) // hb >= 2
        rows = (Sq, Sk, Sk, Sq, Sq, Sq, Sk, Sk)
        bufs = lambda n, extra: [pltpu.VMEM((n + e, S, D), bf16) for S, e in zip(rows, extra + (0,) * 4)]
        sems = lambda n: pltpu.SemaphoreType.DMA((n, 4))
        hbm = pl.BlockSpec(memory_space=pl.ANY)
        outs = pl.pallas_call(
            kernel, grid=(2,), in_specs=[hbm] * 4, out_specs=[hbm] * 4,
            out_shape=[jax.ShapeDtypeStruct((B * H, S, D), bf16) for S in rows[4:]],
            scratch_shapes=bufs(2 * hb, (2, 2, 2, 0)) + bufs(2 * r, (1, 1, 1, 1))
            + [sems(2), sems(2), sems(2 * r + 1), sems(2 * r)]
            + [pltpu.VMEM((Sq // T, Sk, T), bf16), pltpu.VMEM((Sq // T, 8, T), f32),
               pltpu.VMEM((Sk // T, D // 2, T), u32)],
            compiler_params=pltpu.CompilerParams(
                dimension_semantics=("arbitrary",), vmem_limit_bytes=100 * 2**20, disable_bounds_checks=True),
        )(*[x.reshape(B * H, *x.shape[2:]) for x in (q, k, v, do)])
        return tuple(o.reshape(B, H, *o.shape[1:]) for o in outs)

    return mha


_mha = make()


@jax.jit
def pallas_standalone__mha_softmax__near_ridge_kernel(q, k, v, grad_out):
    return _mha(q, k, v, grad_out)
```

```python
import functools
import math

import jax
import jax.numpy as jnp
from jax.experimental import pallas as pl
from jax.experimental.pallas import tpu as pltpu

f32, bf16, u32 = jnp.float32, jnp.bfloat16, jnp.uint32
NN = (((1,), (0,)), ((), ()))
NT = (((1,), (1,)), ((), ()))
T = 128
R = 256
NB = 6


def _dot(a, b, dims=NN):
    return jax.lax.dot_general(a, b, dims, preferred_element_type=f32)


class _Heads:
    def __init__(self, ref, slot):
        self.ref, self.slot, self.shape = ref, slot, ref.shape

    def bitcast(self, dtype):
        return _Heads(self.ref.bitcast(dtype), self.slot)

    def __getitem__(self, i):
        return self.ref[(self.slot(i[0]),) + i[1:]]

    def __setitem__(self, i, x):
        self.ref[(self.slot(i[0]),) + i[1:]] = x


def make(hb=10, r=6, pg=32, tie=2,
         pat="F0_F1_F2_C0_N0_C1_N1_C2_N2_D0_D1_X0_D2_A3_H0_B3_A4_H1_B4_A5_Z3_H2_B5_Y0",
         first="A0_A1_B0_A2_B1_O2_Z0_B2",
         last="F0_F1_F2_C0_N0_C1_N1_C2_N2_O0_D0_D1_X0_O3_D2_H0_H1_H2_O1_Y0_O2"):
    def block(nheads, order, emit, q_ref, k_ref, v_ref, do_ref, o_ref, dq_ref, dk_ref, dv_ref,
              p_carry, r_carry, vT_carry, kT_scr, vT_scr, p_scr, ds_scr):
        Sq, D = q_ref.shape[1:]
        Sk = k_ref.shape[1]
        nq, nk, nr = Sq // T, Sk // T, Sk // R
        scale = D ** -0.5
        c = scale * math.log2(math.e)
        st = {}

        def ld(ref, h, a, n):
            return pltpu.bitcast(ref.bitcast(u32)[h, a // 2:(a + n) // 2, :], bf16)

        def tile_T(ref, h, u):
            return pltpu.bitcast(ld(ref, h, u * T, T).T, u32)

        def pbuf(t):
            return (p_carry, t % nq) if t < nq or t >= nq * nheads else (p_scr, t % NB)

        never = pl.program_id(0) < 0
        taps, pend = [], []

        def tap(xs):
            g = pg // len(xs)
            taps.append([x[(x.shape[0] // g) * a:(x.shape[0] // g) * a + 8] for x in xs for a in range(g)])

        def tied(x):
            while pend and pend[0][0] + tie <= len(taps):
                x = jnp.where(never, pend.pop(0)[1][:x.shape[0]], x)
            return x

        def store_T(ref, h, j, x):
            y = pltpu.bitcast(x.astype(bf16).T, u32)
            ref.bitcast(u32)[h, j * T // 2:(j + 1) * T // 2, :] = y
            pend.append([len(taps), pltpu.bitcast(y[T // 2 - 8:], f32)])

        def A(t):
            h, j = divmod(t, nq)
            qj = ld(q_ref, h, j * T, T)
            mx, xs = None, []
            for u in range(nr):
                s = _dot(ld(k_ref, h, u * R, R), qj, NT)
                xs.append(s)
                for i in range(R // T):
                    st["s", t, u * (R // T) + i] = s[i * T:(i + 1) * T]
                mu = jnp.max(s.reshape(R // 8, 8, T), axis=0)
                mx = mu if mx is None else jnp.maximum(mx, mu)
            st["m", t] = jnp.broadcast_to(jnp.max(mx, axis=0, keepdims=True), (8, T))
            tap(xs[:1])

        def B(t):
            m, ls, tp = tied(st["m", t]), None, taps[-1]
            g = pg // nk
            rows = T // g
            buf, slot = pbuf(t)
            for u in range(nk):
                x = jnp.concatenate([
                    (st["s", t, u][a * rows:(a + 1) * rows].reshape(rows // 8, 8, T)
                     - jnp.where(never, tp[u * g + a], m)[None]).reshape(rows, T) for a in range(g)], axis=0)
                buf[slot, u * T:(u + 1) * T, :] = jnp.exp2(x * c).astype(bf16)
                p = ld(buf, slot, u * T, T).astype(f32)
                lu = jnp.sum(p.reshape(T // 8, 8, T), axis=0)
                ls = lu if ls is None else ls + lu
            st["r", t] = 1.0 / jnp.sum(ls, axis=0, keepdims=True)
            if t >= nq * nheads:
                r_carry[t % nq] = jnp.broadcast_to(st["r", t], (8, T))

        def Z(t):
            if t == nq * nheads:
                for u in range(nk):
                    vT_carry[u] = tile_T(v_ref, nheads, u)

        def F(t):
            h, j = divmod(t, nq)
            if h == 0:
                st["r", t] = r_carry[j][:1]
            doT = do_ref[h, j * T:(j + 1) * T, :].astype(f32).T
            st["doT", t] = doT
            st["do1", t] = (doT * st["r", t]).astype(bf16)
            st["do2", t] = (doT * (st["r", t] * scale)).astype(bf16)

        def C(t):
            h, j = divmod(t, nq)
            if j == 0 and h > 0:
                for u in range(nk):
                    vT_scr[h % 2, u] = tile_T(v_ref, h, u)
            xs = [_dot(pltpu.bitcast(vT_scr[h % 2, u] if h else vT_carry[u], bf16), ld(*pbuf(t), u * T, T))
                  for u in range(nk)]
            st["oT", t] = functools.reduce(jnp.add, xs)
            tap(xs[::4])

        def N(t):
            h, j = divmod(t, nq)
            oT = st["oT", t] * st["r", t]
            store_T(o_ref, h, j, oT)
            st["delta", t] = jnp.sum(oT * st["doT", t], axis=0, keepdims=True) * (st["r", t] * scale)

        def Dd(t):
            delta, xs = tied(st["delta", t]), []
            for u in range(nr):
                dp = _dot(ld(v_ref, t // nq, u * R, R), st["do2", t])
                xs.append(dp)
                p = ld(*pbuf(t), u * R, R).astype(f32)
                ds_scr[t % NB, u * R:(u + 1) * R, :] = (p * (dp - delta)).astype(bf16)
            tap(xs[:1])

        def H(t):
            h, j = divmod(t, nq)
            if j == 0:
                for u in range(nk):
                    kT_scr[h % 2, u] = tile_T(k_ref, h, u)
            xs = [_dot(pltpu.bitcast(kT_scr[h % 2, u], bf16), ld(ds_scr, t % NB, u * T, T)) for u in range(nk)]
            store_T(dq_ref, h, j, functools.reduce(jnp.add, xs))
            tap(xs[::4])

        def key_grad(t, out, buf, ws, dims):
            res = []
            for u in range(nk):
                xs = [_dot(ld(*buf(t + j), u * T, T), ws[j], dims) for j in range(nq)]
                out[t // nq, u * T:(u + 1) * T, :] = functools.reduce(jnp.add, xs).astype(bf16)
                res.append(xs[0])
            tap(res)

        def X(t):
            key_grad(t, dv_ref, pbuf, [st["do1", t + j] for j in range(nq)], NT)

        def Y(t):
            key_grad(t, dk_ref, lambda i: (ds_scr, i % NB), [ld(q_ref, t // nq, j * T, T) for j in range(nq)], NN)

        stages = dict(A=A, B=B, C=C, D=Dd, F=F, H=H, N=N, O=emit, X=X, Y=Y, Z=Z)
        for h in range(max(nheads, 1)):
            for tok in order.split("_"):
                stages[tok[0]](nq * h + int(tok[1:]))

    def kernel(*refs):
        in_hbm, out_hbm = refs[0:4], refs[4:8]
        in_big, out_big, in_sm, out_sm = refs[8:12], refs[12:16], refs[16:20], refs[20:24]
        sem_ib, sem_ob, sem_is, sem_os = refs[24:28]
        carry = refs[28:]
        nh, Sk, D = in_hbm[1].shape
        nb = (nh - 2 * r) // hb
        ahead = (1, 1, 1, 0)
        phase = pl.program_id(0)

        def run(nheads, order, views, emit=None):
            pl.run_scoped(lambda *scr: block(nheads, order, emit, *views, *carry, *scr),
                          pltpu.VMEM((2, Sk // T, D // 2, T), u32), pltpu.VMEM((2, Sk // T, D // 2, T), u32),
                          pltpu.VMEM((NB, Sk, T), bf16), pltpu.VMEM((NB, Sk, T), bf16))

        def run_small(nheads, order, slot, i, emit=None):
            run(nheads, order, [_Heads(x, lambda h: slot + h) for x in in_sm]
                + [_Heads(x, lambda h: i + h) for x in out_sm], emit)

        def copy(hbm, g, buf, pos, n, sem, out):
            a, b = hbm.at[pl.ds(g, n)], buf.at[pl.ds(pos, n)]
            return pltpu.make_async_copy(b, a, sem) if out else pltpu.make_async_copy(a, b, sem)

        def in_b(b):
            return [copy(in_hbm[i], r + b * hb, in_big[i], (b & 1) * (hb + e), hb + e, sem_ib.at[b & 1, i], False)
                    for i, e in enumerate(ahead)]

        def out_b(b):
            return [copy(out_hbm[i], r + b * hb, out_big[i], (b & 1) * hb, hb, sem_ob.at[b & 1, i], True)
                    for i in range(4)]

        def in_s(s, ph, n=1):
            return [copy(in_hbm[i], s + ph * (nh - 2 * r - 1), in_sm[i], s, n, sem_is.at[s, i], False)
                    for i in range(4)]

        def out_s(s, ph, n=1):
            return [copy(out_hbm[i], s + ph * (nh - 2 * r), out_sm[i], s, n, sem_os.at[s, i], True)
                    for i in range(4)]

        def start(cs):
            for x in cs:
                x.start()

        def wait(cs):
            for x in cs:
                x.wait()

        @pl.when(phase == 0)
        def _():
            cs = [x for s in range(r + 1) for x in in_s(s, 0)] + in_b(0)
            start(cs)
            wait(cs[:2])
            run_small(0, first, 0, 0, lambda i: cs[i].wait())
            wait(cs[3:8])

        pl.when(phase == 1)(lambda: wait(in_s(r + 1, 1, r)))

        def small(i, _):
            pl.when((i > 0) & (i < r))(lambda: wait(in_s(i + 1, 0)))
            run_small(1, pat, i + phase, i)
            pl.when(phase == 1)(lambda: start(out_s(i, 1)))
            return 0

        jax.lax.fori_loop(phase * r, phase * (r - 1) + r, small, 0)

        @pl.when(phase == 0)
        def _():
            wait(in_b(0))
            start(in_b(1) + out_s(0, 0, r) + in_s(r + 1, 1, r))

            def big(b, _):
                pl.when(b >= 2)(lambda: wait(out_b(b - 2)))
                pl.when(b >= 1)(lambda: wait(in_b(b)))
                run(hb, pat, [_Heads(x, lambda h, e=e: (b & 1) * (hb + e) + h)
                              for x, e in zip(in_big + out_big, ahead + (0,) * 4)])
                pl.when(b + 2 < nb)(lambda: start(in_b(b + 2)))
                start(out_b(b))
                return 0

            jax.lax.fori_loop(0, nb, big, 0)

        @pl.when(phase == 1)
        def _():
            cs = out_s(2 * r - 1, 1)
            run_small(1, last, 2 * r, 2 * r - 1, lambda i: cs[i].start())
            wait(out_s(0, 0, r) + out_b(nb - 2) + out_b(nb - 1))
            for s in range(r, 2 * r):
                wait(out_s(s, 1))

    @jax.jit
    def mha(q, k, v, do):
        B, H, Sq, D = q.shape
        Sk = k.shape[2]
        assert Sq == 3 * T and r >= 2 and (B * H - 2 * r) % hb == 0 and (B * H - 2 * r) // hb >= 2
        rows = (Sq, Sk, Sk, Sq, Sq, Sq, Sk, Sk)
        bufs = lambda n, extra: [pltpu.VMEM((n + e, S, D), bf16) for S, e in zip(rows, extra + (0,) * 4)]
        sems = lambda n: pltpu.SemaphoreType.DMA((n, 4))
        hbm = pl.BlockSpec(memory_space=pl.ANY)
        outs = pl.pallas_call(
            kernel, grid=(2,), in_specs=[hbm] * 4, out_specs=[hbm] * 4,
            out_shape=[jax.ShapeDtypeStruct((B * H, S, D), bf16) for S in rows[4:]],
            scratch_shapes=bufs(2 * hb, (2, 2, 2, 0)) + bufs(2 * r, (1, 1, 1, 1))
            + [sems(2), sems(2), sems(2 * r + 1), sems(2 * r)]
            + [pltpu.VMEM((Sq // T, Sk, T), bf16), pltpu.VMEM((Sq // T, 8, T), f32),
               pltpu.VMEM((Sk // T, D // 2, T), u32)],
            compiler_params=pltpu.CompilerParams(
                dimension_semantics=("arbitrary",), vmem_limit_bytes=100 * 2**20, disable_bounds_checks=True),
        )(*[x.reshape(B * H, *x.shape[2:]) for x in (q, k, v, do)])
        return tuple(o.reshape(B, H, *o.shape[1:]) for o in outs)

    return mha


_mha = make()


@jax.jit
def pallas_standalone__mha_softmax__near_ridge_kernel(q, k, v, grad_out):
    return _mha(q, k, v, grad_out)
```
